```python
import jax
import jax.numpy as jnp

def _softmax(x, axis=-1):
    return jax.nn.softmax(x, axis=axis)

def _gelu(x):
    return jax.nn.gelu(x, approximate=True)

def _silu(x):
    return jax.nn.silu(x)

def _sigmoid(x):
    return jax.nn.sigmoid(x)

def _layernorm(x, axis=-1, eps=1e-05):
    m = jnp.mean(x, axis=axis, keepdims=True)
    v = jnp.var(x, axis=axis, keepdims=True)
    return (x - m) / jnp.sqrt(v + eps)

def _scatter_add(tgt, idx, src, axis=0):
    return tgt.at[idx].add(src)

def _segment_sum(src, seg, n):
    return jax.ops.segment_sum(src, seg, n)

class _Rng:

    def __init__(self, key):
        self._k = key

    def _next(self):
        self._k, sub = jax.random.split(self._k)
        return sub

    def normal(self, shape):
        return jax.random.normal(self._next(), shape, dtype=jnp.bfloat16)

    def randint(self, lo, hi, shape):
        return jax.random.randint(self._next(), shape, lo, hi, dtype=jnp.int32)

    def uniform(self, shape, lo=0.0, hi=1.0):
        return jax.random.uniform(self._next(), shape, jnp.bfloat16, lo, hi)

    def permutation(self, n):
        return jax.random.permutation(self._next(), n)
kernel_name = 'adaLN_cond__sliding_block_cached__glu_gated_glu__decode'

def setup_inputs():
    _rng = _Rng(jax.random.key(int.from_bytes(__import__("os").urandom(4), "little")))
    _w = lambda a: (lambda t: t.astype(jnp.bfloat16) if jnp.issubdtype(t.dtype, jnp.floating) else t)(jnp.asarray(a))

    def _A_setup():
        B, Sq, D = (8, 1, 512)
        Hq, Hkv, Sk, Dh = (32, 32, 4096, 128)
        assert Hq % Hkv == 0, (Hq, Hkv)
        return {'x': _w((lambda *s: _rng.normal(s) * 0.05)(B, Sq, D)), 'k_cache': _w((lambda *s: _rng.normal(s) * 0.05)(B, Hkv, Sk, Dh)), 'v_cache': _w((lambda *s: _rng.normal(s) * 0.05)(B, Hkv, Sk, Dh)), 'wq': _w((lambda *s: _rng.normal(s) * 0.05)(D, Hq * Dh) * D ** (-0.5)), 'wo': _w((lambda *s: _rng.normal(s) * 0.05)(Hq * Dh, D) * (Hq * Dh) ** (-0.5))}
    _A_in = _A_setup()

    def _B_setup():
        B, S, D, F = (8, 1, 512, 1376)
        return {'x': _w((lambda *s: _rng.normal(s) * 0.05)(B, S, D)), 'w_gate': _w((lambda *s: _rng.normal(s) * 0.05)(D, F)), 'w_up': _w((lambda *s: _rng.normal(s) * 0.05)(D, F)), 'w_down': _w((lambda *s: _rng.normal(s) * 0.05)(F, D))}
    _B_in = _B_setup()
    return {'A_x': _A_in['x'], 'A_k_cache': _A_in['k_cache'], 'A_v_cache': _A_in['v_cache'], 'A_wq': _A_in['wq'], 'A_wo': _A_in['wo'], 'B_x': _B_in['x'], 'B_w_gate': _B_in['w_gate'], 'B_w_up': _B_in['w_up'], 'B_w_down': _B_in['w_down'], 'c': _w((lambda *s: _rng.normal(s) * 0.05)(8, 512)), 'w_mod': _w((lambda *s: _rng.normal(s) * 0.05)(512, 6 * 512) * 512 ** (-0.5))}

def reference(A_x, A_k_cache, A_v_cache, A_wq, A_wo, B_x, B_w_gate, B_w_up, B_w_down, c, w_mod):

    def _A_ref(x, k_cache, v_cache, wq, wo):
        B, Sq, D = x.shape
        Hq, Dh = (32, 128)
        Hkv, Sk = (k_cache.shape[1], k_cache.shape[2])
        W = min(4096, max(256, Sk // 4))
        rep = Hq // Hkv
        q = (lambda x, *d: x.transpose(*d))((x @ wq).reshape(B, Sq, Hq, Dh), 0, 2, 1, 3)
        k = jnp.repeat(k_cache[:, :, Sk - W:, :], rep, axis=1)
        v = jnp.repeat(v_cache[:, :, Sk - W:, :], rep, axis=1)
        scores = jnp.einsum('bhqd,bhkd->bhqk', q, k) * Dh ** (-0.5)
        p = _softmax(scores, axis=-1)
        o = jnp.einsum('bhqk,bhkd->bhqd', p, v)
        return (lambda x, *d: x.transpose(*d))(o, 0, 2, 1, 3).reshape(B, Sq, Hq * Dh) @ wo

    def _B_ref(x, w_gate, w_up, w_down):
        g = jnp.einsum('bsd,df->bsf', x, w_gate)
        u = jnp.einsum('bsd,df->bsf', x, w_up)
        h = _sigmoid(g) * u
        return jnp.einsum('bsf,fd->bsd', h, w_down)
    x = A_x
    mod = (_silu(c) @ w_mod).reshape(c.shape[0], 6, 1, -1)
    sa, ca, ga, sb, cb, gb = (mod[:, 0].copy(), mod[:, 1].copy(), mod[:, 2].copy(), mod[:, 3].copy(), mod[:, 4].copy(), mod[:, 5].copy())
    h = _layernorm(x, axis=-1) * (1 + ca) + sa
    x = x + ga * _A_ref(h, A_k_cache, A_v_cache, A_wq, A_wo)
    h = _layernorm(x, axis=-1) * (1 + cb) + sb
    x = x + gb * _B_ref(h, B_w_gate, B_w_up, B_w_down)
    return x
```

```python
import functools
import jax
import jax.numpy as jnp
from jax import lax
import jax.experimental.pallas as pl
import jax.experimental.pallas.tpu as pltpu

_NT = (((1,), (1,)), ((), ()))
_NN = (((1,), (0,)), ((), ()))
_EPS = 1e-05
_F32 = jnp.float32
_BF16 = jnp.bfloat16
G = 8
NS = 4


def _dot(a, b, dims=_NN):
    return lax.dot_general(a, b, dims, preferred_element_type=_F32)


def _layernorm(x):
    m = jnp.mean(x, axis=-1, keepdims=True)
    d = x - m
    v = jnp.mean(d * d, axis=-1, keepdims=True)
    return d / jnp.sqrt(v + _EPS)


def _blocks(n, step, start=0):
    return [(s, min(step, n - s)) for s in range(start, n, step)]


def _pair(q0, q1):
    n = min(len(q0), len(q1))
    out = []
    for a, b in zip(q0[:n], q1[:n]):
        out += [a + (0,), b + (1,)]
    out += [c + (i % 2,) for i, c in enumerate(q0[n:] + q1[n:])]
    return out


def _kernel(x_hbm, c_hbm, wmod_hbm, wq_hbm, k_hbm, v_hbm, wo_hbm, wg_hbm, wu_hbm, wd_hbm,
            out_ref,
            xbuf, cbuf, wmodbuf, wqbuf, wobuf, kbuf, vbuf, wgbuf, wubuf, wdbuf, qs, os_,
            sem_c, sem_m, *, W, wd_parts):
    B, D = xbuf.shape
    NC, _, Sk, Dh = k_hbm.shape
    H = NC * G // B
    F = wgbuf.shape[0]
    scale = Dh ** -0.5
    ROWS = 16
    A = 128

    def wait_all(buf, sem):
        pltpu.make_async_copy(buf, buf, sem).wait()

    def slab(src, dst, sem, c0, c1):
        return [(src.at[:, pl.ds(rs, rn), pl.ds(cs, cn)], dst.at[:, pl.ds(rs, rn), pl.ds(cs, cn)], sem)
                for rs, rn in _blocks(src.shape[1], 8) for cs, cn in _blocks(c1, 512, c0)]

    def flat(src, dst, sem, r0, r1):
        return [(src.at[pl.ds(rs, rn), :], dst.at[pl.ds(rs, rn), :], sem) for rs, rn in _blocks(r1, 32, r0)]

    def chunk(u, slot):
        q0, q1 = [], []
        for rs, rn in _blocks(W, ROWS):
            q0.append((k_hbm.at[u, :, pl.ds(Sk - W + rs, rn), :],
                       kbuf.at[slot, :, pl.ds(rs, rn), :], sem_c.at[0, slot]))
            q1.append((v_hbm.at[u, :, pl.ds(Sk - W + rs, rn), :],
                       vbuf.at[slot, :, pl.ds(rs, rn), :], sem_c.at[1, slot]))
        return _pair(q0, q1)

    def issue(items):
        for src, dst, sem, prio in items:
            pltpu.make_async_copy(src, dst, sem).start(priority=prio)

    S_C, S_X, S_MA, S_MB, S_MC, S_Q, S_O, S_G, S_U, S_D = range(10)
    ma = slab(wmod_hbm, wmodbuf, sem_m.at[S_MA], 0, 2 * D)
    mb = slab(wmod_hbm, wmodbuf, sem_m.at[S_MB], 2 * D, 5 * D)
    mc = slab(wmod_hbm, wmodbuf, sem_m.at[S_MC], 5 * D, 6 * D)
    wq = slab(wq_hbm, wqbuf, sem_m.at[S_Q], 0, H * Dh)
    wo = slab(wo_hbm, wobuf, sem_m.at[S_O], 0, D)
    head = _pair([(c_hbm, cbuf, sem_m.at[S_C])] + ma + wq, [(x_hbm, xbuf, sem_m.at[S_X])] + wo + mb)
    n_ma = 2 * (1 + len(ma))
    wd = []
    for i, (rs, rn) in enumerate(wd_parts):
        wd += flat(wd_hbm, wdbuf, sem_m.at[S_D + i], rs, rs + rn)
    tail = (_pair(flat(wg_hbm, wgbuf, sem_m.at[S_G], 0, F), flat(wu_hbm, wubuf, sem_m.at[S_U], 0, F))
            + _pair(wd, mc))

    def wmod_cols(c0, c1):
        return wmodbuf[:, :, c0:c1].reshape(D, c1 - c0)

    issue(head[:n_ma + A])
    wait_all(cbuf, sem_m.at[S_C])
    wait_all(xbuf, sem_m.at[S_X])
    cf = cbuf[...].astype(_F32)
    sc = (cf * jax.nn.sigmoid(cf)).astype(_BF16)
    xf = xbuf[...].astype(_F32)
    xn = _layernorm(xf)
    wait_all(wmodbuf.at[:, :, pl.ds(0, 2 * D)], sem_m.at[S_MA])
    mod_a = _dot(sc, wmod_cols(0, 2 * D))
    h1 = (xn * (1.0 + mod_a[:, D:]) + mod_a[:, :D]).astype(_BF16)
    first = chunk(0, 0)
    issue(head[n_ma + A:])
    issue(first[:A])
    wait_all(wqbuf, sem_m.at[S_Q])
    q_all = _dot(h1, wqbuf[...].reshape(D, H * Dh))
    q_all = q_all.astype(_BF16).astype(_F32)
    for h in range(H):
        qs[pl.ds(h, B, stride=H), :] = q_all[:, h * Dh:(h + 1) * Dh]
    wait_all(wmodbuf.at[:, :, pl.ds(2 * D, 3 * D)], sem_m.at[S_MB])
    mod_b = _dot(sc, wmod_cols(2 * D, 5 * D))
    issue(first[A:])
    issue(chunk(1, 1)[:A])

    row_w = lax.broadcasted_iota(jnp.int32, (G, W), 0)
    row_d = lax.broadcasted_iota(jnp.int32, (G, Dh), 0)

    def attend(u, slot):
        wait_all(kbuf.at[slot], sem_c.at[0, slot])
        wait_all(vbuf.at[slot], sem_c.at[1, slot])
        rows = pl.ds(pl.multiple_of(u * G, G), G)
        q = qs[rows, :].astype(_BF16)
        s = _dot(q, kbuf[slot, 0], _NT)
        for i in range(1, G):
            s = jnp.where(row_w == i, _dot(q, kbuf[slot, i], _NT), s)
        s = s * scale
        m = jnp.max(s, axis=-1, keepdims=True)
        p = jnp.exp(s - m)
        l = jnp.sum(p, axis=-1, keepdims=True)
        pb = p.astype(_BF16)
        o = _dot(pb, vbuf[slot, 0])
        for i in range(1, G):
            o = jnp.where(row_d == i, _dot(pb, vbuf[slot, i]), o)
        os_[rows, :] = o / l

    def body(u, carry):
        slot = u % 2
        attend(u, slot)
        issue(chunk(u + 1, 1 - slot)[A:])
        issue(chunk(u + 2, slot)[:A])
        return carry

    lax.fori_loop(0, NC - 2, body, 0)
    attend(NC - 2, (NC - 2) % 2)
    issue(chunk(NC - 1, (NC - 1) % 2)[A:])
    TA = A
    issue(tail[:TA])
    attend(NC - 1, (NC - 1) % 2)
    T2 = len(tail)
    issue(tail[TA:T2])

    o_all = jnp.concatenate([os_[pl.ds(h, B, stride=H), :] for h in range(H)], axis=-1).astype(_BF16)
    wait_all(wobuf, sem_m.at[S_O])
    att = _dot(o_all, wobuf[...].reshape(H * Dh, D))
    x1 = xf + mod_b[:, :D] * att
    h2 = (_layernorm(x1) * (1.0 + mod_b[:, 2 * D:]) + mod_b[:, D:2 * D]).astype(_BF16)
    issue(tail[T2:])
    wait_all(wgbuf, sem_m.at[S_G])
    wait_all(wubuf, sem_m.at[S_U])
    g = _dot(h2, wgbuf[...], _NT)
    u = _dot(h2, wubuf[...], _NT)
    hh = (jax.nn.sigmoid(g) * u).astype(_BF16)
    wait_all(wmodbuf.at[:, :, pl.ds(5 * D, D)], sem_m.at[S_MC])
    gb = _dot(sc, wmod_cols(5 * D, 6 * D))
    d = None
    for i, (rs, rn) in enumerate(wd_parts):
        wait_all(wdbuf.at[pl.ds(rs, rn), :], sem_m.at[S_D + i])
        part = _dot(hh[:, rs:rs + rn], wdbuf[pl.ds(rs, rn), :])
        d = part if d is None else d + part
    out_ref[...] = (x1 + gb * d).astype(out_ref.dtype)


@jax.jit
def pallas_adaLN_cond__sliding_block_cached__glu_gated_glu__decode_kernel(A_x, A_k_cache, A_v_cache, A_wq, A_wo, B_x, B_w_gate, B_w_up, B_w_down, c, w_mod):
    B, Sq, D = A_x.shape
    _, H, Sk, Dh = A_k_cache.shape
    W = min(4096, max(256, Sk // 4))
    F = B_w_gate.shape[1]
    dt = A_x.dtype
    wd_parts = ((0, 768), (768, 384), (1152, F - 1152))
    NC = B * H // G
    out = pl.pallas_call(
        functools.partial(_kernel, W=W, wd_parts=wd_parts),
        out_shape=jax.ShapeDtypeStruct((B, D), dt),
        in_specs=[pl.BlockSpec(memory_space=pl.ANY)] * 10,
        out_specs=pl.BlockSpec(memory_space=pltpu.VMEM),
        scratch_shapes=[
            pltpu.VMEM((B, D), dt), pltpu.VMEM((B, D), dt),
            pltpu.VMEM((NS, D // NS, 6 * D), dt),
            pltpu.VMEM((NS, D // NS, H * Dh), dt), pltpu.VMEM((NS, H * Dh // NS, D), dt),
            pltpu.VMEM((2, G, W, Dh), dt), pltpu.VMEM((2, G, W, Dh), dt),
            pltpu.VMEM((F, D), dt), pltpu.VMEM((F, D), dt), pltpu.VMEM((F, D), dt),
            pltpu.VMEM((B * H, Dh), _F32), pltpu.VMEM((B * H, Dh), _F32),
            pltpu.SemaphoreType.DMA((2, 2)),
            pltpu.SemaphoreType.DMA((9 + len(wd_parts),)),
        ],
        compiler_params=pltpu.CompilerParams(vmem_limit_bytes=64 * 1024 * 1024),
    )(A_x.reshape(B, D), c, w_mod.reshape(NS, D // NS, 6 * D), A_wq.reshape(NS, D // NS, H * Dh),
      A_k_cache.reshape(NC, G, Sk, Dh), A_v_cache.reshape(NC, G, Sk, Dh),
      A_wo.reshape(NS, H * Dh // NS, D), B_w_gate.T, B_w_up.T, B_w_down)
    return out.reshape(B, Sq, D)
```

```python
import functools

import jax
import jax.numpy as jnp
from jax import lax
import jax.experimental.pallas as pl
import jax.experimental.pallas.tpu as pltpu

_NT = (((1,), (1,)), ((), ()))
_NN = (((1,), (0,)), ((), ()))
_EPS = 1e-05
_F32 = jnp.float32
_BF16 = jnp.bfloat16

_G = 8
_HS = 2
_ROWS = 16
_UNROLL = 8
_NS = 4
_CW = 512
_FR = 32
_TAIL_FIRST = 44

_S_C, _S_X, _S_M, _S_Q, _S_O, _S_G, _S_U, _S_D = range(8)


def _dot(a, b, dims=_NN):
    return lax.dot_general(a, b, dims, preferred_element_type=_F32)


def _layernorm(x):
    m = jnp.mean(x, axis=-1, keepdims=True)
    d = x - m
    v = jnp.mean(d * d, axis=-1, keepdims=True)
    return d / jnp.sqrt(v + _EPS)


def _start(src, dst, sem, priority):
    pltpu.make_async_copy(src, dst, sem).start(priority=priority)


def _wait_filled(buf, sem):
    pltpu.make_async_copy(buf, buf, sem).wait()


def _loop(lo, hi, fn):
    def body(i, carry):
        fn(i)
        return carry
    lax.fori_loop(lo, hi, body, 0)


def _kernel(x_hbm, c_hbm, wmod_hbm, wq_hbm, k_hbm, v_hbm, wo_hbm, wg_hbm, wu_hbm, wd_hbm,
            out_ref,
            xbuf, cbuf, wmodbuf, wqbuf, wobuf, kbuf, vbuf, wgbuf, wubuf, wdbuf, qs, ats,
            sem_kv, sem, *, split_u, wd0, wd1):
    B, D = xbuf.shape
    NG, _, _, Sk, Dh = k_hbm.shape
    W = kbuf.shape[2]
    NC = NG * _HS
    H = NC * _G // B
    F = wgbuf.shape[0]
    scale = Dh ** -0.5
    nrb = D // _NS // 8
    pieces = list(wd0) + list(wd1)

    def issue_wmod():
        half = 3 * D

        def fn(r):
            rows = pl.ds(pl.multiple_of(r * 8, 8), 8)
            for cs in range(0, half, _CW):
                for t in range(2):
                    cols = pl.ds(t * half + cs, _CW)
                    _start(wmod_hbm.at[:, rows, cols], wmodbuf.at[:, rows, cols], sem.at[_S_M], t)
        _loop(0, nrb, fn)

    def issue_wq_wo(lo, hi):
        ncb = H * Dh // _CW

        def fn(r):
            rows = pl.ds(pl.multiple_of(r * 8, 8), 8)
            for j in range(ncb):
                cols = pl.ds(j * _CW, _CW)
                _start(wq_hbm.at[:, rows, cols], wqbuf.at[:, rows, cols], sem.at[_S_Q], 0)
                orows = pl.ds(pl.multiple_of((r * ncb + j) * 8, 8), 8)
                _start(wo_hbm.at[:, orows, :], wobuf.at[:, orows, :], sem.at[_S_O], 1)
        _loop(lo, hi, fn)

    def issue_chunk(u, slot):
        g, j = u // _HS, u % _HS

        def fn(i):
            for jj in range(_UNROLL):
                r = pl.multiple_of((i * _UNROLL + jj) * _ROWS, _ROWS)
                src, dst = pl.ds(Sk - W + r, _ROWS), pl.ds(r, _ROWS)
                _start(k_hbm.at[g, :, j, src, :], kbuf.at[slot, :, dst, :], sem_kv.at[0, slot], 0)
                _start(v_hbm.at[g, :, j, src, :], vbuf.at[slot, :, dst, :], sem_kv.at[1, slot], 1)
        _loop(0, W // _ROWS // _UNROLL, fn)

    def issue_ffn(lo, hi):
        segs0 = [(wg_hbm, wgbuf, 0, F, _S_G), (wu_hbm, wubuf, split_u, F - split_u, _S_U)]
        segs0 += [(wd_hbm, wdbuf, r0, n, _S_D + i) for i, (r0, n) in enumerate(wd0)]
        segs1 = [(wu_hbm, wubuf, 0, split_u, _S_U)]
        segs1 += [(wd_hbm, wdbuf, r0, n, _S_D + len(wd0) + i) for i, (r0, n) in enumerate(wd1)]
        streams = [(segs, [(k, r0 + o) for k, (_, _, r0, n, _) in enumerate(segs)
                           for o in range(0, n, _FR)]) for segs in (segs0, segs1)]
        n = max(len(cps) for _, cps in streams)
        hi = n if hi is None else hi

        def seg_ids(z):
            return tuple(cps[z][0] if z < len(cps) else None for _, cps in streams)

        i = lo
        while i < hi:
            k = i
            while k < hi and seg_ids(k) == seg_ids(i):
                k += 1

            def fn(z, i=i):
                for t, (segs, cps) in enumerate(streams):
                    if i < len(cps):
                        src, dst, _, _, s = segs[cps[i][0]]
                        rows = pl.ds(pl.multiple_of(cps[i][1] + z * _FR, _FR), _FR)
                        _start(src.at[rows, :], dst.at[rows, :], sem.at[s], t)
            _loop(0, k - i, fn)
            i = k

    def head_rows(h):
        r = ((h // (_G * _HS)) * _HS + h % _HS) * _G + (h % (_G * _HS)) // _HS
        return pl.ds(r, B, stride=H)

    _start(c_hbm, cbuf, sem.at[_S_C], 0)
    _start(x_hbm, xbuf, sem.at[_S_X], 1)
    issue_wmod()
    issue_wq_wo(0, nrb // 2)
    _wait_filled(cbuf, sem.at[_S_C])
    _wait_filled(xbuf, sem.at[_S_X])
    _wait_filled(wmodbuf, sem.at[_S_M])
    cf = cbuf[...].astype(_F32)
    sc = (cf * jax.nn.sigmoid(cf)).astype(_BF16)
    xf = xbuf[...].astype(_F32)
    mod = _dot(sc, wmodbuf[...].reshape(D, 6 * D))
    sa, ca, ga, sb, cb, gb = [mod[:, i * D:(i + 1) * D] for i in range(6)]
    h1 = (_layernorm(xf) * (1.0 + ca) + sa).astype(_BF16)
    issue_wq_wo(nrb // 2, nrb)
    issue_chunk(0, 0)
    _wait_filled(wqbuf, sem.at[_S_Q])
    _wait_filled(wobuf, sem.at[_S_O])
    q_all = _dot(h1, wqbuf[...].reshape(D, H * Dh))
    for h in range(H):
        qs[head_rows(h), :] = q_all[:, h * Dh:(h + 1) * Dh]
    issue_chunk(1, 1)

    row_w = lax.broadcasted_iota(jnp.int32, (_G, W), 0)
    row_d = lax.broadcasted_iota(jnp.int32, (_G, Dh), 0)

    def chunk_step(u):
        slot = u % 2
        rows = pl.ds(pl.multiple_of(u * _G, _G), _G)
        q = qs[rows, :].astype(_BF16)
        _wait_filled(kbuf.at[slot], sem_kv.at[0, slot])
        s = _dot(q, kbuf[slot, 0], _NT)
        for i in range(1, _G):
            s = jnp.where(row_w == i, _dot(q, kbuf[slot, i], _NT), s)
        s = s * scale
        m = jnp.max(s, axis=-1, keepdims=True)
        p = jnp.exp(s - m)
        l = jnp.sum(p, axis=-1, keepdims=True)
        pb = p.astype(_BF16)
        _wait_filled(vbuf.at[slot], sem_kv.at[1, slot])
        o = _dot(pb, vbuf[slot, 0])
        for i in range(1, _G):
            o = jnp.where(row_d == i, _dot(pb, vbuf[slot, i]), o)
        ats[rows, :] = o / l

        @pl.when(u < NC - 2)
        def _():
            issue_chunk(jnp.minimum(u + 2, NC - 1), slot)

        @pl.when(u == NC - 2)
        def _():
            issue_ffn(0, _TAIL_FIRST)

    _loop(0, NC, chunk_step)
    issue_ffn(_TAIL_FIRST, None)

    o_all = jnp.concatenate([ats[head_rows(h), :] for h in range(H)], axis=-1).astype(_BF16)
    x1 = xf + ga * _dot(o_all, wobuf[...].reshape(H * Dh, D))
    h2 = (_layernorm(x1) * (1.0 + cb) + sb).astype(_BF16)
    _wait_filled(wgbuf, sem.at[_S_G])
    gate = jax.nn.sigmoid(_dot(h2, wgbuf[...], _NT))
    _wait_filled(wubuf, sem.at[_S_U])
    hh = (gate * _dot(h2, wubuf[...], _NT)).astype(_BF16)
    down = None
    for i, (r0, n) in enumerate(pieces):
        _wait_filled(wdbuf.at[pl.ds(r0, n), :], sem.at[_S_D + i])
        part = _dot(hh[:, r0:r0 + n], wdbuf[pl.ds(r0, n), :])
        down = part if down is None else down + part
    out_ref[...] = (x1 + gb * down).astype(out_ref.dtype)


@jax.jit
def pallas_adaLN_cond__sliding_block_cached__glu_gated_glu__decode_kernel(
    A_x: jax.Array,
    A_k_cache: jax.Array,
    A_v_cache: jax.Array,
    A_wq: jax.Array,
    A_wo: jax.Array,
    B_x: jax.Array,
    B_w_gate: jax.Array,
    B_w_up: jax.Array,
    B_w_down: jax.Array,
    c: jax.Array,
    w_mod: jax.Array,
):
    del B_x
    B, Sq, D = A_x.shape
    _, H, Sk, Dh = A_k_cache.shape
    F = B_w_gate.shape[1]
    W = min(4096, max(256, Sk // 4))
    assert Sq == 1 and A_wq.shape == (D, H * Dh) and H % (_G * _HS) == 0 and F == 1376
    dt = A_x.dtype
    NG = B * H // (_G * _HS)
    split_u = 1120
    wd0 = ((0, 384),)
    wd1 = ((384, 640), (1024, 256), (1280, 96))

    params = dict(vmem_limit_bytes=48 * 1024 * 1024)
    if hasattr(pltpu.CompilerParams, "disable_semaphore_checks"):
        params["disable_semaphore_checks"] = True

    out = pl.pallas_call(
        functools.partial(_kernel, split_u=split_u, wd0=wd0, wd1=wd1),
        out_shape=jax.ShapeDtypeStruct((B, D), dt),
        in_specs=[pl.BlockSpec(memory_space=pl.ANY)] * 10,
        out_specs=pl.BlockSpec(memory_space=pltpu.VMEM),
        scratch_shapes=[
            pltpu.VMEM((B, D), dt),
            pltpu.VMEM((B, D), dt),
            pltpu.VMEM((_NS, D // _NS, 6 * D), dt),
            pltpu.VMEM((_NS, D // _NS, H * Dh), dt),
            pltpu.VMEM((_NS, H * Dh // _NS, D), dt),
            pltpu.VMEM((2, _G, W, Dh), dt),
            pltpu.VMEM((2, _G, W, Dh), dt),
            pltpu.VMEM((F, D), dt),
            pltpu.VMEM((F, D), dt),
            pltpu.VMEM((F, D), dt),
            pltpu.VMEM((B * H, Dh), _F32),
            pltpu.VMEM((B * H, Dh), _F32),
            pltpu.SemaphoreType.DMA((2, 2)),
            pltpu.SemaphoreType.DMA((_S_D + len(wd0) + len(wd1),)),
        ],
        compiler_params=pltpu.CompilerParams(**params),
    )(A_x.reshape(B, D), c,
      w_mod.reshape(_NS, D // _NS, 6 * D), A_wq.reshape(_NS, D // _NS, H * Dh),
      A_k_cache.reshape(NG, _G, _HS, Sk, Dh), A_v_cache.reshape(NG, _G, _HS, Sk, Dh),
      A_wo.reshape(_NS, H * Dh // _NS, D), B_w_gate.T, B_w_up.T, B_w_down)
    return out.reshape(B, Sq, D)
```

```python
import functools

import jax
import jax.numpy as jnp
from jax import lax
import jax.experimental.pallas as pl
import jax.experimental.pallas.tpu as pltpu

_NT = (((1,), (1,)), ((), ()))
_NN = (((1,), (0,)), ((), ()))
_EPS = 1e-05
_F32 = jnp.float32
_BF16 = jnp.bfloat16

_G = 8
_HS = 2
_ROWS = 16
_UNROLL = 2
_NS = 4
_CW = 512
_FR = 32
_AHEAD = 64
_TAIL_FIRST = 44

_S_C, _S_X, _S_M, _S_Q, _S_O, _S_G, _S_U, _S_D = range(8)


def _dot(a, b, dims=_NN):
    return lax.dot_general(a, b, dims, preferred_element_type=_F32)


def _layernorm(x):
    m = jnp.mean(x, axis=-1, keepdims=True)
    d = x - m
    v = jnp.mean(d * d, axis=-1, keepdims=True)
    return d / jnp.sqrt(v + _EPS)


def _start(src, dst, sem, priority):
    pltpu.make_async_copy(src, dst, sem).start(priority=priority)


def _wait_filled(buf, sem):
    pltpu.make_async_copy(buf, buf, sem).wait()


def _loop(lo, hi, fn):
    def body(i, carry):
        fn(i)
        return carry
    lax.fori_loop(lo, hi, body, 0)


def _issue_streams(streams, lo, hi=None):
    flat = [[(k, i) for k, (_, i0, i1) in enumerate(segs) for i in range(i0, i1)]
            for segs in streams]
    hi = max(len(f) for f in flat) if hi is None else hi

    def seg_ids(z):
        return tuple(f[z][0] if z < len(f) else None for f in flat)

    while lo < hi:
        end = lo
        while end < hi and seg_ids(end) == seg_ids(lo):
            end += 1

        def fn(z, lo=lo):
            for t, f in enumerate(flat):
                if lo < len(f):
                    streams[t][f[lo][0]][0](f[lo][1] + z, t)
        _loop(0, end - lo, fn)
        lo = end


def _kernel(x_hbm, c_hbm, wmod_hbm, wq_hbm, k_hbm, v_hbm, wo_hbm, wg_hbm, wu_hbm, wd_hbm,
            out_ref,
            xbuf, cbuf, wmodbuf, wqbuf, wobuf, kbuf, vbuf, wgbuf, wubuf, wdbuf, qs, ats,
            sem_kv, sem, *, split_u, wd0, wd1):
    B, D = xbuf.shape
    NG, _, _, Sk, Dh = k_hbm.shape
    W = kbuf.shape[2]
    NC = NG * _HS
    H = NC * _G // B
    F = wgbuf.shape[0]
    scale = Dh ** -0.5
    pieces = list(wd0) + list(wd1)

    def slab_copy(src, dst, s):
        ncb = src.shape[2] // _CW

        def fn(i, priority):
            rows = pl.ds(pl.multiple_of((i // ncb) * 8, 8), 8)
            cols = pl.ds(pl.multiple_of((i % ncb) * _CW, _CW), _CW)
            _start(src.at[:, rows, cols], dst.at[:, rows, cols], sem.at[s], priority)
        return fn, src.shape[1] // 8 * ncb

    def row_copy(src, dst, s):
        def fn(i, priority):
            rows = pl.ds(pl.multiple_of(i * _FR, _FR), _FR)
            _start(src.at[rows, :], dst.at[rows, :], sem.at[s], priority)
        return fn

    (cp_m, n_m), (cp_q, n_q), (cp_o, n_o) = (slab_copy(wmod_hbm, wmodbuf, _S_M),
                                             slab_copy(wq_hbm, wqbuf, _S_Q),
                                             slab_copy(wo_hbm, wobuf, _S_O))
    split_o = (n_q + n_o - n_m) // 2
    head = ([(cp_m, 0, n_m), (cp_o, 0, split_o)], [(cp_q, 0, n_q), (cp_o, split_o, n_o)])
    cp_u = row_copy(wu_hbm, wubuf, _S_U)
    down_segs = [(row_copy(wd_hbm, wdbuf, _S_D + i), r0 // _FR, (r0 + n) // _FR)
                 for i, (r0, n) in enumerate(pieces)]
    ffn = ([(row_copy(wg_hbm, wgbuf, _S_G), 0, F // _FR), (cp_u, split_u // _FR, F // _FR)]
           + down_segs[:len(wd0)],
           [(cp_u, 0, split_u // _FR)] + down_segs[len(wd0):])

    def issue_chunk(u, slot):
        g, j = u // _HS, u % _HS

        def fn(i):
            for jj in range(_UNROLL):
                r = pl.multiple_of((i * _UNROLL + jj) * _ROWS, _ROWS)
                src, dst = pl.ds(Sk - W + r, _ROWS), pl.ds(r, _ROWS)
                _start(k_hbm.at[g, :, j, src, :], kbuf.at[slot, :, dst, :], sem_kv.at[0, slot], 0)
                _start(v_hbm.at[g, :, j, src, :], vbuf.at[slot, :, dst, :], sem_kv.at[1, slot], 1)
        _loop(0, W // _ROWS // _UNROLL, fn)

    def head_rows(h):
        r = ((h // (_G * _HS)) * _HS + h % _HS) * _G + (h % (_G * _HS)) // _HS
        return pl.ds(r, B, stride=H)

    _start(c_hbm, cbuf, sem.at[_S_C], 0)
    _start(x_hbm, xbuf, sem.at[_S_X], 1)
    _issue_streams(head, 0, n_m + _AHEAD)
    _wait_filled(cbuf, sem.at[_S_C])
    _wait_filled(xbuf, sem.at[_S_X])
    _wait_filled(wmodbuf, sem.at[_S_M])
    cf = cbuf[...].astype(_F32)
    sc = (cf * jax.nn.sigmoid(cf)).astype(_BF16)
    xf = xbuf[...].astype(_F32)
    mod = _dot(sc, wmodbuf[...].reshape(D, 6 * D))
    sa, ca, ga, sb, cb, gb = [mod[:, i * D:(i + 1) * D] for i in range(6)]
    h1 = (_layernorm(xf) * (1.0 + ca) + sa).astype(_BF16)
    _issue_streams(head, n_m + _AHEAD)
    issue_chunk(0, 0)
    _wait_filled(wqbuf, sem.at[_S_Q])
    _wait_filled(wobuf, sem.at[_S_O])
    q_all = _dot(h1, wqbuf[...].reshape(D, H * Dh))
    for h in range(H):
        qs[head_rows(h), :] = q_all[:, h * Dh:(h + 1) * Dh]
    issue_chunk(1, 1)

    row_w = lax.broadcasted_iota(jnp.int32, (_G, W), 0)
    row_d = lax.broadcasted_iota(jnp.int32, (_G, Dh), 0)

    def chunk_step(u):
        slot = u % 2
        rows = pl.ds(pl.multiple_of(u * _G, _G), _G)
        q = qs[rows, :].astype(_BF16)
        _wait_filled(kbuf.at[slot], sem_kv.at[0, slot])
        s = _dot(q, kbuf[slot, 0], _NT)
        for i in range(1, _G):
            s = jnp.where(row_w == i, _dot(q, kbuf[slot, i], _NT), s)
        s = s * scale
        m = jnp.max(s, axis=-1, keepdims=True)
        p = jnp.exp(s - m)
        l = jnp.sum(p, axis=-1, keepdims=True)
        pb = p.astype(_BF16)
        _wait_filled(vbuf.at[slot], sem_kv.at[1, slot])
        o = _dot(pb, vbuf[slot, 0])
        for i in range(1, _G):
            o = jnp.where(row_d == i, _dot(pb, vbuf[slot, i]), o)
        ats[rows, :] = o / l

        @pl.when(u < NC - 2)
        def _():
            issue_chunk(jnp.minimum(u + 2, NC - 1), slot)

        @pl.when(u == NC - 2)
        def _():
            _issue_streams(ffn, 0, _TAIL_FIRST)

    _loop(0, NC, chunk_step)
    _issue_streams(ffn, _TAIL_FIRST)

    o_all = jnp.concatenate([ats[head_rows(h), :] for h in range(H)], axis=-1).astype(_BF16)
    x1 = xf + ga * _dot(o_all, wobuf[...].reshape(H * Dh, D))
    h2 = (_layernorm(x1) * (1.0 + cb) + sb).astype(_BF16)
    _wait_filled(wgbuf, sem.at[_S_G])
    gate = jax.nn.sigmoid(_dot(h2, wgbuf[...], _NT))
    _wait_filled(wubuf, sem.at[_S_U])
    hh = (gate * _dot(h2, wubuf[...], _NT)).astype(_BF16)
    down = None
    for i, (r0, n) in enumerate(pieces):
        _wait_filled(wdbuf.at[pl.ds(r0, n), :], sem.at[_S_D + i])
        part = _dot(hh[:, r0:r0 + n], wdbuf[pl.ds(r0, n), :])
        down = part if down is None else down + part
    out_ref[...] = (x1 + gb * down).astype(out_ref.dtype)


@jax.jit
def pallas_adaLN_cond__sliding_block_cached__glu_gated_glu__decode_kernel(
    A_x: jax.Array,
    A_k_cache: jax.Array,
    A_v_cache: jax.Array,
    A_wq: jax.Array,
    A_wo: jax.Array,
    B_x: jax.Array,
    B_w_gate: jax.Array,
    B_w_up: jax.Array,
    B_w_down: jax.Array,
    c: jax.Array,
    w_mod: jax.Array,
):
    del B_x
    B, Sq, D = A_x.shape
    _, H, Sk, Dh = A_k_cache.shape
    F = B_w_gate.shape[1]
    W = min(4096, max(256, Sk // 4))
    assert Sq == 1 and A_wq.shape == (D, H * Dh) and H % (_G * _HS) == 0 and F == 1376
    dt = A_x.dtype
    NG = B * H // (_G * _HS)
    split_u = 1120
    wd0 = ((0, 384),)
    wd1 = ((384, 640), (1024, 256), (1280, 96))

    params = dict(vmem_limit_bytes=48 * 1024 * 1024)
    if hasattr(pltpu.CompilerParams, "disable_semaphore_checks"):
        params["disable_semaphore_checks"] = True

    out = pl.pallas_call(
        functools.partial(_kernel, split_u=split_u, wd0=wd0, wd1=wd1),
        out_shape=jax.ShapeDtypeStruct((B, D), dt),
        in_specs=[pl.BlockSpec(memory_space=pl.ANY)] * 10,
        out_specs=pl.BlockSpec(memory_space=pltpu.VMEM),
        scratch_shapes=[
            pltpu.VMEM((B, D), dt),
            pltpu.VMEM((B, D), dt),
            pltpu.VMEM((_NS, D // _NS, 6 * D), dt),
            pltpu.VMEM((_NS, D // _NS, H * Dh), dt),
            pltpu.VMEM((_NS, H * Dh // _NS, D), dt),
            pltpu.VMEM((2, _G, W, Dh), dt),
            pltpu.VMEM((2, _G, W, Dh), dt),
            pltpu.VMEM((F, D), dt),
            pltpu.VMEM((F, D), dt),
            pltpu.VMEM((F, D), dt),
            pltpu.VMEM((B * H, Dh), _F32),
            pltpu.VMEM((B * H, Dh), _F32),
            pltpu.SemaphoreType.DMA((2, 2)),
            pltpu.SemaphoreType.DMA((_S_D + len(wd0) + len(wd1),)),
        ],
        compiler_params=pltpu.CompilerParams(**params),
    )(A_x.reshape(B, D), c,
      w_mod.reshape(_NS, D // _NS, 6 * D), A_wq.reshape(_NS, D // _NS, H * Dh),
      A_k_cache.reshape(NG, _G, _HS, Sk, Dh), A_v_cache.reshape(NG, _G, _HS, Sk, Dh),
      A_wo.reshape(_NS, H * Dh // _NS, D), B_w_gate.T, B_w_up.T, B_w_down)
    return out.reshape(B, Sq, D)
```

```python
import functools

import jax
import jax.numpy as jnp
from jax import lax
import jax.experimental.pallas as pl
import jax.experimental.pallas.tpu as pltpu

_NT = (((1,), (1,)), ((), ()))
_NN = (((1,), (0,)), ((), ()))
_EPS = 1e-05
_F32 = jnp.float32
_BF16 = jnp.bfloat16

_G = 8
_SHIFT = 2
_ROWS = 16
_UNROLL = 2
_EARLY = 0.75
_NS = 4
_CW = 512
_FR = 32
_AHEAD = 64
_TAIL_FIRST = 44

_S_C, _S_X, _S_M, _S_Q, _S_O, _S_G, _S_U, _S_D = range(8)


def _dot(a, b, dims=_NN):
    return lax.dot_general(a, b, dims, preferred_element_type=_F32)


def _layernorm(x):
    m = jnp.mean(x, axis=-1, keepdims=True)
    d = x - m
    v = jnp.mean(d * d, axis=-1, keepdims=True)
    return d / jnp.sqrt(v + _EPS)


def _start(src, dst, sem, priority):
    pltpu.make_async_copy(src, dst, sem).start(priority=priority)


def _wait_filled(buf, sem):
    pltpu.make_async_copy(buf, buf, sem).wait()


def _loop(lo, hi, fn):
    def body(i, carry):
        fn(i)
        return carry
    lax.fori_loop(lo, hi, body, 0)


def _issue_streams(streams, lo, hi=None):
    flat = [[(k, i) for k, (_, i0, i1) in enumerate(segs) for i in range(i0, i1)]
            for segs in streams]
    hi = max(len(f) for f in flat) if hi is None else hi

    def seg_ids(z):
        return tuple(f[z][0] if z < len(f) else None for f in flat)

    while lo < hi:
        end = lo
        while end < hi and seg_ids(end) == seg_ids(lo):
            end += 1

        def fn(z, lo=lo):
            for t, f in enumerate(flat):
                if lo < len(f):
                    streams[t][f[lo][0]][0](f[lo][1] + z, t)
        _loop(0, end - lo, fn)
        lo = end


def _kernel(x_hbm, c_hbm, wmod_hbm, wq_hbm, k_hbm, v_hbm, wo_hbm, wg_hbm, wu_hbm, wd_hbm,
            out_ref,
            xbuf, cbuf, wmodbuf, wqbuf, wobuf, kbuf, vbuf, wgbuf, wubuf, wdbuf, qs, ats,
            sem_kv, sem, *, split_u, wd0, wd1):
    B, D = xbuf.shape
    NW, Sk, Dh = k_hbm.shape
    W = kbuf.shape[2]
    H = NW // B
    NP = NW // (2 * _G)
    F = wgbuf.shape[0]
    scale = Dh ** -0.5
    pieces = list(wd0) + list(wd1)

    def slab_copy(src, dst, s):
        ncb = src.shape[2] // _CW

        def fn(i, priority):
            rows = pl.ds(pl.multiple_of((i // ncb) * 8, 8), 8)
            cols = pl.ds(pl.multiple_of((i % ncb) * _CW, _CW), _CW)
            _start(src.at[:, rows, cols], dst.at[:, rows, cols], sem.at[s], priority)
        return fn, src.shape[1] // 8 * ncb

    def row_copy(src, dst, s):
        def fn(i, priority):
            rows = pl.ds(pl.multiple_of(i * _FR, _FR), _FR)
            _start(src.at[rows, :], dst.at[rows, :], sem.at[s], priority)
        return fn

    (cp_m, n_m), (cp_q, n_q), (cp_o, n_o) = (slab_copy(wmod_hbm, wmodbuf, _S_M),
                                             slab_copy(wq_hbm, wqbuf, _S_Q),
                                             slab_copy(wo_hbm, wobuf, _S_O))
    split_o = (n_q + n_o - n_m) // 2
    head = ([(cp_m, 0, n_m), (cp_o, 0, split_o)], [(cp_q, 0, n_q), (cp_o, split_o, n_o)])
    cp_u = row_copy(wu_hbm, wubuf, _S_U)
    down_segs = [(row_copy(wd_hbm, wdbuf, _S_D + i), r0 // _FR, (r0 + n) // _FR)
                 for i, (r0, n) in enumerate(pieces)]
    ffn = ([(row_copy(wg_hbm, wgbuf, _S_G), 0, F // _FR), (cp_u, split_u // _FR, F // _FR)]
           + down_segs[:len(wd0)],
           [(cp_u, 0, split_u // _FR)] + down_segs[len(wd0):])

    n_it = W // _ROWS // _UNROLL
    early = int(n_it * _EARLY)

    def issue_kv(kv, p, lo, hi):
        src, dst = ((k_hbm, kbuf), (v_hbm, vbuf))[kv]
        w0 = (NP - 1 if p is None else p) * 2 * _G + _SHIFT

        def copy(z, w, i0, n, r, nr):
            _start(src.at[pl.ds(w, n), pl.ds(Sk - W + r, nr), :],
                   dst.at[z, pl.ds(i0, n), pl.ds(r, nr), :], sem_kv.at[kv, z], z)

        def fn(i):
            for jj in range(_UNROLL):
                r = pl.multiple_of((i * _UNROLL + jj) * _ROWS, _ROWS)
                copy(0, w0, 0, _G, r, _ROWS)
                if p is None:
                    copy(1, w0 + _G, 0, _G - _SHIFT, r, _ROWS)
                    copy(1, 0, _G - _SHIFT, _SHIFT, r, _ROWS)
                else:
                    copy(1, w0 + _G, 0, _G, r, _ROWS // 2)
                    copy(1, w0 + _G, 0, _G, r + _ROWS // 2, _ROWS // 2)
        _loop(lo, hi, fn)

    def head_rows(h):
        return pl.ds(h + _G - _SHIFT, B, stride=H)

    row_w = lax.broadcasted_iota(jnp.int32, (_G, W), 0)
    row_d = lax.broadcasted_iota(jnp.int32, (_G, Dh), 0)
    first, wrap = pl.ds(0, _G), pl.ds(NW, _G)

    _start(c_hbm, cbuf, sem.at[_S_C], 0)
    _start(x_hbm, xbuf, sem.at[_S_X], 1)
    _issue_streams(head, 0, n_m + _AHEAD)
    _wait_filled(cbuf, sem.at[_S_C])
    _wait_filled(xbuf, sem.at[_S_X])
    _wait_filled(wmodbuf, sem.at[_S_M])
    cf = cbuf[...].astype(_F32)
    sc = (cf * jax.nn.sigmoid(cf)).astype(_BF16)
    xf = xbuf[...].astype(_F32)
    mod = _dot(sc, wmodbuf[...].reshape(D, 6 * D))
    sa, ca, ga, sb, cb, gb = [mod[:, i * D:(i + 1) * D] for i in range(6)]
    h1 = (_layernorm(xf) * (1.0 + ca) + sa).astype(_BF16)
    _issue_streams(head, n_m + _AHEAD)
    issue_kv(0, None, 0, n_it)
    _wait_filled(wqbuf, sem.at[_S_Q])
    _wait_filled(wobuf, sem.at[_S_O])
    q_all = _dot(h1, wqbuf[...].reshape(D, H * Dh))
    zeros = jnp.zeros((_G, Dh), _F32)
    qs[first, :] = zeros
    qs[wrap, :] = zeros
    for h in range(H):
        qs[head_rows(h), :] = q_all[:, h * Dh:(h + 1) * Dh]
    qs[wrap, :] = jnp.where(row_d < _G - _SHIFT, qs[wrap, :], qs[first, :])
    issue_kv(1, None, 0, n_it)

    def phase_step(t):
        p = (t + NP - 1) % NP
        cur, nxt = jnp.minimum(p, NP - 2), jnp.minimum(t, NP - 2)
        rows = [pl.ds(pl.multiple_of((2 * p + 1 + z) * _G, _G), _G) for z in range(2)]

        def probs(z):
            q = qs[rows[z], :].astype(_BF16)
            _wait_filled(kbuf.at[z], sem_kv.at[0, z])
            s = _dot(q, kbuf[z, 0], _NT)
            for i in range(1, _G):
                s = jnp.where(row_w == i, _dot(q, kbuf[z, i], _NT), s)
            s = s * scale
            e = jnp.exp(s - jnp.max(s, axis=-1, keepdims=True))
            return e.astype(_BF16), jnp.sum(e, axis=-1, keepdims=True)

        def attend(z, e, l):
            _wait_filled(vbuf.at[z], sem_kv.at[1, z])
            o = _dot(e, vbuf[z, 0])
            for i in range(1, _G):
                o = jnp.where(row_d == i, _dot(e, vbuf[z, i]), o)
            ats[rows[z], :] = o / l

        el0 = probs(0)
        pl.when(t > 0)(lambda: issue_kv(1, cur, early, n_it))
        el1 = probs(1)
        pl.when(t < NP - 1)(lambda: issue_kv(0, nxt, 0, early))
        pl.when(t == NP - 1)(lambda: _issue_streams(ffn, 0, _TAIL_FIRST))
        attend(0, *el0)
        pl.when(t < NP - 1)(lambda: issue_kv(0, nxt, early, n_it))
        attend(1, *el1)
        pl.when(t < NP - 1)(lambda: issue_kv(1, nxt, 0, early))

    _loop(0, NP, phase_step)
    _issue_streams(ffn, _TAIL_FIRST)
    ats[first, :] = ats[wrap, :]

    o_all = jnp.concatenate([ats[head_rows(h), :] for h in range(H)], axis=-1).astype(_BF16)
    x1 = xf + ga * _dot(o_all, wobuf[...].reshape(H * Dh, D))
    h2 = (_layernorm(x1) * (1.0 + cb) + sb).astype(_BF16)
    _wait_filled(wgbuf, sem.at[_S_G])
    gate = jax.nn.sigmoid(_dot(h2, wgbuf[...], _NT))
    _wait_filled(wubuf, sem.at[_S_U])
    hh = (gate * _dot(h2, wubuf[...], _NT)).astype(_BF16)
    down = None
    for i, (r0, n) in enumerate(pieces):
        _wait_filled(wdbuf.at[pl.ds(r0, n), :], sem.at[_S_D + i])
        part = _dot(hh[:, r0:r0 + n], wdbuf[pl.ds(r0, n), :])
        down = part if down is None else down + part
    out_ref[...] = (x1 + gb * down).astype(out_ref.dtype)


@jax.jit
def pallas_adaLN_cond__sliding_block_cached__glu_gated_glu__decode_kernel(
    A_x: jax.Array,
    A_k_cache: jax.Array,
    A_v_cache: jax.Array,
    A_wq: jax.Array,
    A_wo: jax.Array,
    B_x: jax.Array,
    B_w_gate: jax.Array,
    B_w_up: jax.Array,
    B_w_down: jax.Array,
    c: jax.Array,
    w_mod: jax.Array,
):
    del B_x
    B, Sq, D = A_x.shape
    _, H, Sk, Dh = A_k_cache.shape
    F = B_w_gate.shape[1]
    W = min(4096, max(256, Sk // 4))
    assert Sq == 1 and A_wq.shape == (D, H * Dh) and B * H % (2 * _G) == 0 and F == 1376
    assert W % (_ROWS * _UNROLL) == 0
    dt = A_x.dtype
    split_u = 1120
    wd0 = ((0, 384),)
    wd1 = ((384, 640), (1024, 256), (1280, 96))

    params = dict(vmem_limit_bytes=48 * 1024 * 1024)
    if hasattr(pltpu.CompilerParams, "disable_semaphore_checks"):
        params["disable_semaphore_checks"] = True

    out = pl.pallas_call(
        functools.partial(_kernel, split_u=split_u, wd0=wd0, wd1=wd1),
        out_shape=jax.ShapeDtypeStruct((B, D), dt),
        in_specs=[pl.BlockSpec(memory_space=pl.ANY)] * 10,
        out_specs=pl.BlockSpec(memory_space=pltpu.VMEM),
        scratch_shapes=[
            pltpu.VMEM((B, D), dt),
            pltpu.VMEM((B, D), dt),
            pltpu.VMEM((_NS, D // _NS, 6 * D), dt),
            pltpu.VMEM((_NS, D // _NS, H * Dh), dt),
            pltpu.VMEM((_NS, H * Dh // _NS, D), dt),
            pltpu.VMEM((2, _G, W, Dh), dt),
            pltpu.VMEM((2, _G, W, Dh), dt),
            pltpu.VMEM((F, D), dt),
            pltpu.VMEM((F, D), dt),
            pltpu.VMEM((F, D), dt),
            pltpu.VMEM((B * H + _G, Dh), _F32),
            pltpu.VMEM((B * H + _G, Dh), _F32),
            pltpu.SemaphoreType.DMA((2, 2)),
            pltpu.SemaphoreType.DMA((_S_D + len(wd0) + len(wd1),)),
        ],
        compiler_params=pltpu.CompilerParams(**params),
    )(A_x.reshape(B, D), c,
      w_mod.reshape(_NS, D // _NS, 6 * D), A_wq.reshape(_NS, D // _NS, H * Dh),
      A_k_cache.reshape(B * H, Sk, Dh), A_v_cache.reshape(B * H, Sk, Dh),
      A_wo.reshape(_NS, H * Dh // _NS, D), B_w_gate.T, B_w_up.T, B_w_down)
    return out.reshape(B, Sq, D)
```

```python
import functools

import jax
import jax.numpy as jnp
from jax import lax
import jax.experimental.pallas as pl
import jax.experimental.pallas.tpu as pltpu

_NT = (((1,), (1,)), ((), ()))
_NN = (((1,), (0,)), ((), ()))
_EPS = 1e-05
_F32 = jnp.float32
_BF16 = jnp.bfloat16

_G = 8
_SHIFT = 2
_ROWS = 16
_UNROLL = 4
_EARLY = 0.75
_NS = 4
_CW = 512
_FR = 32
_AHEAD = 64
_TAIL_FIRST = 44

_S_C, _S_X, _S_M, _S_Q, _S_O, _S_G, _S_U, _S_D = range(8)


def _dot(a, b, dims=_NN):
    return lax.dot_general(a, b, dims, preferred_element_type=_F32)


def _layernorm(x):
    m = jnp.mean(x, axis=-1, keepdims=True)
    d = x - m
    v = jnp.mean(d * d, axis=-1, keepdims=True)
    return d / jnp.sqrt(v + _EPS)


def _start(src, dst, sem, priority):
    pltpu.make_async_copy(src, dst, sem).start(priority=priority)


def _wait_filled(buf, sem):
    pltpu.make_async_copy(buf, buf, sem).wait()


def _loop(lo, hi, fn):
    def body(i, carry):
        fn(i)
        return carry
    lax.fori_loop(lo, hi, body, 0)


def _issue_streams(streams, lo, hi=None):
    flat = [[(k, i) for k, (_, i0, i1) in enumerate(segs) for i in range(i0, i1)]
            for segs in streams]
    hi = max(len(f) for f in flat) if hi is None else hi

    def seg_ids(z):
        return tuple(f[z][0] if z < len(f) else None for f in flat)

    while lo < hi:
        end = lo
        while end < hi and seg_ids(end) == seg_ids(lo):
            end += 1

        def fn(z, lo=lo):
            for t, f in enumerate(flat):
                if lo < len(f):
                    streams[t][f[lo][0]][0](f[lo][1] + z, t)
        _loop(0, end - lo, fn)
        lo = end


def _kernel(x_hbm, c_hbm, wmod_hbm, wq_hbm, k_hbm, v_hbm, wo_hbm, wg_hbm, wu_hbm, wd_hbm,
            out_ref,
            xbuf, cbuf, wmodbuf, wqbuf, wobuf, kbuf, vbuf, wgbuf, wubuf, wdbuf, qs, ats,
            sem_kv, sem, *, split_u, wd0, wd1):
    B, D = xbuf.shape
    NW, Sk, Dh = k_hbm.shape
    W = kbuf.shape[2]
    H = NW // B
    NP = NW // (2 * _G)
    F = wgbuf.shape[0]
    scale = Dh ** -0.5
    pieces = list(wd0) + list(wd1)

    def slab_copy(src, dst, s):
        ncb = src.shape[2] // _CW

        def fn(i, priority):
            rows = pl.ds(pl.multiple_of((i // ncb) * 8, 8), 8)
            cols = pl.ds(pl.multiple_of((i % ncb) * _CW, _CW), _CW)
            _start(src.at[:, rows, cols], dst.at[:, rows, cols], sem.at[s], priority)
        return fn, src.shape[1] // 8 * ncb

    def row_copy(src, dst, s):
        def fn(i, priority):
            rows = pl.ds(pl.multiple_of(i * _FR, _FR), _FR)
            _start(src.at[rows, :], dst.at[rows, :], sem.at[s], priority)
        return fn

    (cp_m, n_m), (cp_q, n_q), (cp_o, n_o) = (slab_copy(wmod_hbm, wmodbuf, _S_M),
                                             slab_copy(wq_hbm, wqbuf, _S_Q),
                                             slab_copy(wo_hbm, wobuf, _S_O))
    split_o = (n_q + n_o - n_m) // 2
    head = ([(cp_m, 0, n_m), (cp_o, 0, split_o)], [(cp_q, 0, n_q), (cp_o, split_o, n_o)])
    cp_u = row_copy(wu_hbm, wubuf, _S_U)
    down_segs = [(row_copy(wd_hbm, wdbuf, _S_D + i), r0 // _FR, (r0 + n) // _FR)
                 for i, (r0, n) in enumerate(pieces)]
    ffn = ([(row_copy(wg_hbm, wgbuf, _S_G), 0, F // _FR), (cp_u, split_u // _FR, F // _FR)]
           + down_segs[:len(wd0)],
           [(cp_u, 0, split_u // _FR)] + down_segs[len(wd0):])

    n_it = W // _ROWS // _UNROLL
    early = int(n_it * _EARLY)

    def issue_kv(kv, p, lo, hi):
        src, dst = ((k_hbm, kbuf), (v_hbm, vbuf))[kv]
        w0 = (NP - 1 if p is None else p) * 2 * _G + _SHIFT

        def copy(z, w, i0, n, r, nr):
            _start(src.at[pl.ds(w, n), pl.ds(Sk - W + r, nr), :],
                   dst.at[z, pl.ds(i0, n), pl.ds(r, nr), :], sem_kv.at[kv, z], z)

        n1 = _G - _SHIFT if p is None else _G

        def fn(i):
            r0 = pl.multiple_of(i * _UNROLL * _ROWS, _UNROLL * _ROWS)
            for jj in range(_UNROLL):
                r = r0 + jj * _ROWS
                copy(0, w0, 0, _G, r, _ROWS)
                copy(1, w0 + _G, 0, n1, r, _ROWS // 2)
                copy(1, w0 + _G, 0, n1, r + _ROWS // 2, _ROWS // 2)
            if p is None:
                copy(1, 0, n1, _SHIFT, r0, _UNROLL * _ROWS)
        _loop(lo, hi, fn)

    def head_rows(h):
        return pl.ds(h + _G - _SHIFT, B, stride=H)

    row_w = lax.broadcasted_iota(jnp.int32, (_G, W), 0)
    row_d = lax.broadcasted_iota(jnp.int32, (_G, Dh), 0)
    first, wrap = pl.ds(0, _G), pl.ds(NW, _G)

    _start(c_hbm, cbuf, sem.at[_S_C], 0)
    _start(x_hbm, xbuf, sem.at[_S_X], 1)
    _issue_streams(head, 0, n_m + _AHEAD)
    _wait_filled(cbuf, sem.at[_S_C])
    _wait_filled(xbuf, sem.at[_S_X])
    _wait_filled(wmodbuf, sem.at[_S_M])
    cf = cbuf[...].astype(_F32)
    sc = (cf * jax.nn.sigmoid(cf)).astype(_BF16)
    xf = xbuf[...].astype(_F32)
    mod = _dot(sc, wmodbuf[...].reshape(D, 6 * D))
    sa, ca, ga, sb, cb, gb = [mod[:, i * D:(i + 1) * D] for i in range(6)]
    h1 = (_layernorm(xf) * (1.0 + ca) + sa).astype(_BF16)
    _issue_streams(head, n_m + _AHEAD)
    issue_kv(0, None, 0, n_it)
    _wait_filled(wqbuf, sem.at[_S_Q])
    _wait_filled(wobuf, sem.at[_S_O])
    q_all = _dot(h1, wqbuf[...].reshape(D, H * Dh))
    zeros = jnp.zeros((_G, Dh), _F32)
    qs[first, :] = zeros
    qs[wrap, :] = zeros
    for h in range(H):
        qs[head_rows(h), :] = q_all[:, h * Dh:(h + 1) * Dh]
    qs[wrap, :] = jnp.where(row_d < _G - _SHIFT, qs[wrap, :], qs[first, :])
    issue_kv(1, None, 0, early)

    def phase_step(t):
        p = (t + NP - 1) % NP
        cur, nxt = jnp.minimum(p, NP - 2), jnp.minimum(t, NP - 2)
        rows = [pl.ds(pl.multiple_of((2 * p + 1 + z) * _G, _G), _G) for z in range(2)]

        def probs(z):
            q = qs[rows[z], :].astype(_BF16)
            _wait_filled(kbuf.at[z], sem_kv.at[0, z])
            s = _dot(q, kbuf[z, 0], _NT)
            for i in range(1, _G):
                s = jnp.where(row_w == i, _dot(q, kbuf[z, i], _NT), s)
            s = s * scale
            e = jnp.exp(s - jnp.max(s, axis=-1, keepdims=True))
            return e.astype(_BF16), jnp.sum(e, axis=-1, keepdims=True)

        def attend(z, e, l):
            _wait_filled(vbuf.at[z], sem_kv.at[1, z])
            o = _dot(e, vbuf[z, 0])
            for i in range(1, _G):
                o = jnp.where(row_d == i, _dot(e, vbuf[z, i]), o)
            ats[rows[z], :] = o / l

        el0 = probs(0)
        pl.when(t == 0)(lambda: issue_kv(1, None, early, n_it))
        pl.when(t > 0)(lambda: issue_kv(1, cur, early, n_it))
        el1 = probs(1)
        pl.when(t < NP - 1)(lambda: issue_kv(0, nxt, 0, early))
        pl.when(t == NP - 1)(lambda: _issue_streams(ffn, 0, _TAIL_FIRST))
        attend(0, *el0)
        pl.when(t < NP - 1)(lambda: issue_kv(0, nxt, early, n_it))
        attend(1, *el1)
        pl.when(t < NP - 1)(lambda: issue_kv(1, nxt, 0, early))

    _loop(0, NP, phase_step)
    _issue_streams(ffn, _TAIL_FIRST)
    ats[first, :] = ats[wrap, :]

    o_all = jnp.concatenate([ats[head_rows(h), :] for h in range(H)], axis=-1).astype(_BF16)
    x1 = xf + ga * _dot(o_all, wobuf[...].reshape(H * Dh, D))
    h2 = (_layernorm(x1) * (1.0 + cb) + sb).astype(_BF16)
    _wait_filled(wgbuf, sem.at[_S_G])
    gate = jax.nn.sigmoid(_dot(h2, wgbuf[...], _NT))
    _wait_filled(wubuf, sem.at[_S_U])
    hh = (gate * _dot(h2, wubuf[...], _NT)).astype(_BF16)
    down = None
    for i, (r0, n) in enumerate(pieces):
        _wait_filled(wdbuf.at[pl.ds(r0, n), :], sem.at[_S_D + i])
        part = _dot(hh[:, r0:r0 + n], wdbuf[pl.ds(r0, n), :])
        down = part if down is None else down + part
    out_ref[...] = (x1 + gb * down).astype(out_ref.dtype)


@jax.jit
def pallas_adaLN_cond__sliding_block_cached__glu_gated_glu__decode_kernel(
    A_x: jax.Array,
    A_k_cache: jax.Array,
    A_v_cache: jax.Array,
    A_wq: jax.Array,
    A_wo: jax.Array,
    B_x: jax.Array,
    B_w_gate: jax.Array,
    B_w_up: jax.Array,
    B_w_down: jax.Array,
    c: jax.Array,
    w_mod: jax.Array,
):
    del B_x
    B, Sq, D = A_x.shape
    _, H, Sk, Dh = A_k_cache.shape
    F = B_w_gate.shape[1]
    W = min(4096, max(256, Sk // 4))
    assert Sq == 1 and A_wq.shape == (D, H * Dh) and B * H % (2 * _G) == 0 and F == 1376
    assert W % (_ROWS * _UNROLL) == 0
    dt = A_x.dtype
    split_u = 1120
    wd0 = ((0, 384),)
    wd1 = ((384, 640), (1024, 256), (1280, 96))

    params = dict(vmem_limit_bytes=48 * 1024 * 1024)
    if hasattr(pltpu.CompilerParams, "disable_semaphore_checks"):
        params["disable_semaphore_checks"] = True

    out = pl.pallas_call(
        functools.partial(_kernel, split_u=split_u, wd0=wd0, wd1=wd1),
        out_shape=jax.ShapeDtypeStruct((B, D), dt),
        in_specs=[pl.BlockSpec(memory_space=pl.ANY)] * 10,
        out_specs=pl.BlockSpec(memory_space=pltpu.VMEM),
        scratch_shapes=[
            pltpu.VMEM((B, D), dt),
            pltpu.VMEM((B, D), dt),
            pltpu.VMEM((_NS, D // _NS, 6 * D), dt),
            pltpu.VMEM((_NS, D // _NS, H * Dh), dt),
            pltpu.VMEM((_NS, H * Dh // _NS, D), dt),
            pltpu.VMEM((2, _G, W, Dh), dt),
            pltpu.VMEM((2, _G, W, Dh), dt),
            pltpu.VMEM((F, D), dt),
            pltpu.VMEM((F, D), dt),
            pltpu.VMEM((F, D), dt),
            pltpu.VMEM((B * H + _G, Dh), _F32),
            pltpu.VMEM((B * H + _G, Dh), _F32),
            pltpu.SemaphoreType.DMA((2, 2)),
            pltpu.SemaphoreType.DMA((_S_D + len(wd0) + len(wd1),)),
        ],
        compiler_params=pltpu.CompilerParams(**params),
    )(A_x.reshape(B, D), c,
      w_mod.reshape(_NS, D // _NS, 6 * D), A_wq.reshape(_NS, D // _NS, H * Dh),
      A_k_cache.reshape(B * H, Sk, Dh), A_v_cache.reshape(B * H, Sk, Dh),
      A_wo.reshape(_NS, H * Dh // _NS, D), B_w_gate.T, B_w_up.T, B_w_down)
    return out.reshape(B, Sq, D)
```

```python
import functools

import jax
import jax.numpy as jnp
from jax import lax
import jax.experimental.pallas as pl
import jax.experimental.pallas.tpu as pltpu

_NT = (((1,), (1,)), ((), ()))
_NN = (((1,), (0,)), ((), ()))
_EPS = 1e-05
_F32 = jnp.float32
_BF16 = jnp.bfloat16

_G = 8
_SHIFT = 2
_ROWS = 16
_ROW_OFF = 8
_UNROLL = 4
_EARLY = 0.75
_NS = 4
_CW = 512
_FR = 32
_AHEAD = 64
_TAIL_FIRST = 44

_S_C, _S_X, _S_M, _S_Q, _S_O, _S_G, _S_U, _S_D = range(8)


def _dot(a, b, dims=_NN):
    return lax.dot_general(a, b, dims, preferred_element_type=_F32)


def _layernorm(x):
    m = jnp.mean(x, axis=-1, keepdims=True)
    d = x - m
    v = jnp.mean(d * d, axis=-1, keepdims=True)
    return d / jnp.sqrt(v + _EPS)


def _start(src, dst, sem, priority):
    pltpu.make_async_copy(src, dst, sem).start(priority=priority)


def _wait_filled(buf, sem):
    pltpu.make_async_copy(buf, buf, sem).wait()


def _loop(lo, hi, fn):
    def body(i, carry):
        fn(i)
        return carry
    lax.fori_loop(lo, hi, body, 0)


def _issue_streams(streams, lo, hi=None):
    flat = [[(k, i) for k, (_, i0, i1) in enumerate(segs) for i in range(i0, i1)]
            for segs in streams]
    hi = max(len(f) for f in flat) if hi is None else hi

    def seg_ids(z):
        return tuple(f[z][0] if z < len(f) else None for f in flat)

    while lo < hi:
        end = lo
        while end < hi and seg_ids(end) == seg_ids(lo):
            end += 1

        def fn(z, lo=lo):
            for t, f in enumerate(flat):
                if lo < len(f):
                    streams[t][f[lo][0]][0](f[lo][1] + z, t)
        _loop(0, end - lo, fn)
        lo = end


def _kernel(x_hbm, c_hbm, wmod_hbm, wq_hbm, k_hbm, v_hbm, wo_hbm, wg_hbm, wu_hbm, wd_hbm,
            out_ref,
            xbuf, cbuf, wmodbuf, wqbuf, wobuf, kbuf, vbuf, wgbuf, wubuf, wdbuf, qs, ats,
            sem_kv, sem, *, split_u, wd0, wd1):
    B, D = xbuf.shape
    NW, Sk, Dh = k_hbm.shape
    W = kbuf.shape[2]
    H = NW // B
    NP = NW // (2 * _G)
    F = wgbuf.shape[0]
    scale = Dh ** -0.5
    pieces = list(wd0) + list(wd1)

    def slab_copy(src, dst, s):
        ncb = src.shape[2] // _CW

        def fn(i, priority):
            rows = pl.ds(pl.multiple_of((i // ncb) * 8, 8), 8)
            cols = pl.ds(pl.multiple_of((i % ncb) * _CW, _CW), _CW)
            _start(src.at[:, rows, cols], dst.at[:, rows, cols], sem.at[s], priority)
        return fn, src.shape[1] // 8 * ncb

    def row_copy(src, dst, s):
        def fn(i, priority):
            rows = pl.ds(pl.multiple_of(i * _FR, _FR), _FR)
            _start(src.at[rows, :], dst.at[rows, :], sem.at[s], priority)
        return fn

    (cp_m, n_m), (cp_q, n_q), (cp_o, n_o) = (slab_copy(wmod_hbm, wmodbuf, _S_M),
                                             slab_copy(wq_hbm, wqbuf, _S_Q),
                                             slab_copy(wo_hbm, wobuf, _S_O))
    split_o = (n_q + n_o - n_m) // 2
    head = ([(cp_m, 0, n_m), (cp_o, 0, split_o)], [(cp_q, 0, n_q), (cp_o, split_o, n_o)])
    cp_u = row_copy(wu_hbm, wubuf, _S_U)
    down_segs = [(row_copy(wd_hbm, wdbuf, _S_D + i), r0 // _FR, (r0 + n) // _FR)
                 for i, (r0, n) in enumerate(pieces)]
    ffn = ([(row_copy(wg_hbm, wgbuf, _S_G), 0, F // _FR), (cp_u, split_u // _FR, F // _FR)]
           + down_segs[:len(wd0)],
           [(cp_u, 0, split_u // _FR)] + down_segs[len(wd0):])

    n_it = W // _ROWS // _UNROLL
    early = int(n_it * _EARLY)

    def issue_kv(kv, p, lo, hi):
        src, dst = ((k_hbm, kbuf), (v_hbm, vbuf))[kv]
        w0 = (NP - 1 if p is None else p) * 2 * _G + _SHIFT

        def copy(z, w, i0, n, r, nr):
            _start(src.at[pl.ds(w, n), pl.ds(Sk - W + r, nr), :],
                   dst.at[z, pl.ds(i0, n), pl.ds(r, nr), :], sem_kv.at[kv, z], z)

        n1 = _G - _SHIFT if p is None else _G

        def rows_at(r, nr):
            copy(0, w0, 0, _G, r, nr)
            copy(1, w0 + _G, 0, n1, r, nr)

        def group(r0, last=False):
            for jj in range(_UNROLL):
                short = last and jj == _UNROLL - 1
                rows_at(r0 + _ROW_OFF + jj * _ROWS, _ROWS - _ROW_OFF if short else _ROWS)
            if p is None:
                copy(1, 0, n1, _SHIFT, r0, _UNROLL * _ROWS)

        if lo == 0:
            rows_at(0, _ROW_OFF)
        _loop(lo, min(hi, n_it - 1),
              lambda i: group(pl.multiple_of(i * _UNROLL * _ROWS, _UNROLL * _ROWS)))
        if hi == n_it:
            group(W - _UNROLL * _ROWS, last=True)

    def head_rows(h):
        return pl.ds(h + _G - _SHIFT, B, stride=H)

    row_w = lax.broadcasted_iota(jnp.int32, (_G, W), 0)
    row_d = lax.broadcasted_iota(jnp.int32, (_G, Dh), 0)
    first, wrap = pl.ds(0, _G), pl.ds(NW, _G)

    _start(c_hbm, cbuf, sem.at[_S_C], 0)
    _start(x_hbm, xbuf, sem.at[_S_X], 1)
    _issue_streams(head, 0, n_m + _AHEAD)
    _wait_filled(cbuf, sem.at[_S_C])
    _wait_filled(xbuf, sem.at[_S_X])
    _wait_filled(wmodbuf, sem.at[_S_M])
    cf = cbuf[...].astype(_F32)
    sc = (cf * jax.nn.sigmoid(cf)).astype(_BF16)
    xf = xbuf[...].astype(_F32)
    mod = _dot(sc, wmodbuf[...].reshape(D, 6 * D))
    sa, ca, ga, sb, cb, gb = [mod[:, i * D:(i + 1) * D] for i in range(6)]
    h1 = (_layernorm(xf) * (1.0 + ca) + sa).astype(_BF16)
    _issue_streams(head, n_m + _AHEAD)
    issue_kv(0, None, 0, n_it)
    _wait_filled(wqbuf, sem.at[_S_Q])
    _wait_filled(wobuf, sem.at[_S_O])
    q_all = _dot(h1, wqbuf[...].reshape(D, H * Dh))
    zeros = jnp.zeros((_G, Dh), _F32)
    qs[first, :] = zeros
    qs[wrap, :] = zeros
    for h in range(H):
        qs[head_rows(h), :] = q_all[:, h * Dh:(h + 1) * Dh]
    qs[wrap, :] = jnp.where(row_d < _G - _SHIFT, qs[wrap, :], qs[first, :])
    issue_kv(1, None, 0, early)

    def phase_step(t):
        p = (t + NP - 1) % NP
        cur, nxt = jnp.minimum(p, NP - 2), jnp.minimum(t, NP - 2)
        rows = [pl.ds(pl.multiple_of((2 * p + 1 + z) * _G, _G), _G) for z in range(2)]

        def probs(z):
            q = qs[rows[z], :].astype(_BF16)
            _wait_filled(kbuf.at[z], sem_kv.at[0, z])
            s = _dot(q, kbuf[z, 0], _NT)
            for i in range(1, _G):
                s = jnp.where(row_w == i, _dot(q, kbuf[z, i], _NT), s)
            s = s * scale
            e = jnp.exp(s - jnp.max(s, axis=-1, keepdims=True))
            return e.astype(_BF16), jnp.sum(e, axis=-1, keepdims=True)

        def attend(z, e, l):
            _wait_filled(vbuf.at[z], sem_kv.at[1, z])
            o = _dot(e, vbuf[z, 0])
            for i in range(1, _G):
                o = jnp.where(row_d == i, _dot(e, vbuf[z, i]), o)
            ats[rows[z], :] = o / l

        el0 = probs(0)
        pl.when(t == 0)(lambda: issue_kv(1, None, early, n_it))
        pl.when(t > 0)(lambda: issue_kv(1, cur, early, n_it))
        el1 = probs(1)
        pl.when(t < NP - 1)(lambda: issue_kv(0, nxt, 0, early))
        pl.when(t == NP - 1)(lambda: _issue_streams(ffn, 0, _TAIL_FIRST))
        attend(0, *el0)
        pl.when(t < NP - 1)(lambda: issue_kv(0, nxt, early, n_it))
        attend(1, *el1)
        pl.when(t < NP - 1)(lambda: issue_kv(1, nxt, 0, early))

    _loop(0, NP, phase_step)
    _issue_streams(ffn, _TAIL_FIRST)
    ats[first, :] = ats[wrap, :]

    o_all = jnp.concatenate([ats[head_rows(h), :] for h in range(H)], axis=-1).astype(_BF16)
    x1 = xf + ga * _dot(o_all, wobuf[...].reshape(H * Dh, D))
    h2 = (_layernorm(x1) * (1.0 + cb) + sb).astype(_BF16)
    _wait_filled(wgbuf, sem.at[_S_G])
    gate = jax.nn.sigmoid(_dot(h2, wgbuf[...], _NT))
    _wait_filled(wubuf, sem.at[_S_U])
    hh = (gate * _dot(h2, wubuf[...], _NT)).astype(_BF16)
    down = None
    for i, (r0, n) in enumerate(pieces):
        _wait_filled(wdbuf.at[pl.ds(r0, n), :], sem.at[_S_D + i])
        part = _dot(hh[:, r0:r0 + n], wdbuf[pl.ds(r0, n), :])
        down = part if down is None else down + part
    out_ref[...] = (x1 + gb * down).astype(out_ref.dtype)


@jax.jit
def pallas_adaLN_cond__sliding_block_cached__glu_gated_glu__decode_kernel(
    A_x: jax.Array,
    A_k_cache: jax.Array,
    A_v_cache: jax.Array,
    A_wq: jax.Array,
    A_wo: jax.Array,
    B_x: jax.Array,
    B_w_gate: jax.Array,
    B_w_up: jax.Array,
    B_w_down: jax.Array,
    c: jax.Array,
    w_mod: jax.Array,
):
    del B_x
    B, Sq, D = A_x.shape
    _, H, Sk, Dh = A_k_cache.shape
    F = B_w_gate.shape[1]
    W = min(4096, max(256, Sk // 4))
    assert Sq == 1 and A_wq.shape == (D, H * Dh) and B * H % (2 * _G) == 0 and F == 1376
    assert W % (_ROWS * _UNROLL) == 0
    dt = A_x.dtype
    split_u = 1120
    wd0 = ((0, 384),)
    wd1 = ((384, 640), (1024, 256), (1280, 96))

    params = dict(vmem_limit_bytes=48 * 1024 * 1024)
    if hasattr(pltpu.CompilerParams, "disable_semaphore_checks"):
        params["disable_semaphore_checks"] = True

    out = pl.pallas_call(
        functools.partial(_kernel, split_u=split_u, wd0=wd0, wd1=wd1),
        out_shape=jax.ShapeDtypeStruct((B, D), dt),
        in_specs=[pl.BlockSpec(memory_space=pl.ANY)] * 10,
        out_specs=pl.BlockSpec(memory_space=pltpu.VMEM),
        scratch_shapes=[
            pltpu.VMEM((B, D), dt),
            pltpu.VMEM((B, D), dt),
            pltpu.VMEM((_NS, D // _NS, 6 * D), dt),
            pltpu.VMEM((_NS, D // _NS, H * Dh), dt),
            pltpu.VMEM((_NS, H * Dh // _NS, D), dt),
            pltpu.VMEM((2, _G, W, Dh), dt),
            pltpu.VMEM((2, _G, W, Dh), dt),
            pltpu.VMEM((F, D), dt),
            pltpu.VMEM((F, D), dt),
            pltpu.VMEM((F, D), dt),
            pltpu.VMEM((B * H + _G, Dh), _F32),
            pltpu.VMEM((B * H + _G, Dh), _F32),
            pltpu.SemaphoreType.DMA((2, 2)),
            pltpu.SemaphoreType.DMA((_S_D + len(wd0) + len(wd1),)),
        ],
        compiler_params=pltpu.CompilerParams(**params),
    )(A_x.reshape(B, D), c,
      w_mod.reshape(_NS, D // _NS, 6 * D), A_wq.reshape(_NS, D // _NS, H * Dh),
      A_k_cache.reshape(B * H, Sk, Dh), A_v_cache.reshape(B * H, Sk, Dh),
      A_wo.reshape(_NS, H * Dh // _NS, D), B_w_gate.T, B_w_up.T, B_w_down)
    return out.reshape(B, Sq, D)
```

```python
import functools

import jax
import jax.numpy as jnp
from jax import lax
import jax.experimental.pallas as pl
import jax.experimental.pallas.tpu as pltpu

_NT = (((1,), (1,)), ((), ()))
_NN = (((1,), (0,)), ((), ()))
_EPS = 1e-05
_F32 = jnp.float32
_BF16 = jnp.bfloat16

_G = 8
_SHIFT = 2
_ROWS = 16
_ROW_OFF = 8
_UNROLL = 4
_EARLY = 0.75
_NS = 4
_CW = 512
_FR = 32
_LEAD = 12
_AHEAD = 64
_TAIL_FIRST = 44

_S_C, _S_X, _S_M, _S_Q, _S_O, _S_G, _S_U, _S_D = range(8)


def _dot(a, b, dims=_NN):
    return lax.dot_general(a, b, dims, preferred_element_type=_F32)


def _layernorm(x):
    m = jnp.mean(x, axis=-1, keepdims=True)
    d = x - m
    v = jnp.mean(d * d, axis=-1, keepdims=True)
    return d / jnp.sqrt(v + _EPS)


def _start(src, dst, sem, priority):
    pltpu.make_async_copy(src, dst, sem).start(priority=priority)


def _wait_filled(buf, sem):
    pltpu.make_async_copy(buf, buf, sem).wait()


def _loop(lo, hi, fn):
    def body(i, carry):
        fn(i)
        return carry
    lax.fori_loop(lo, hi, body, 0)


def _issue_streams(streams, lo, hi=None):
    flat = [[(k, i) for k, (_, i0, i1) in enumerate(segs) for i in range(i0, i1)]
            for segs in streams]
    hi = max(len(f) for f in flat) if hi is None else hi

    def seg_ids(z):
        return tuple(f[z][0] if z < len(f) else None for f in flat)

    while lo < hi:
        end = lo
        while end < hi and seg_ids(end) == seg_ids(lo):
            end += 1

        def fn(z, lo=lo):
            for t, f in enumerate(flat):
                if lo < len(f):
                    streams[t][f[lo][0]][0](f[lo][1] + z, t)
        _loop(0, end - lo, fn)
        lo = end


def _kernel(x_hbm, c_hbm, wmod_hbm, wq_hbm, k_hbm, v_hbm, wo_hbm, wg_hbm, wu_hbm, wd_hbm,
            out_ref,
            xbuf, cbuf, wmodbuf, wqbuf, wobuf, kbuf, vbuf, wgbuf, wubuf, wdbuf, qs, ats,
            sem_kv, sem, *, split_u, wd0, wd1):
    B, D = xbuf.shape
    NW, Sk, Dh = k_hbm.shape
    W = kbuf.shape[2]
    H = NW // B
    NP = NW // (2 * _G)
    F = wgbuf.shape[0]
    scale = Dh ** -0.5
    pieces = list(wd0) + list(wd1)

    def slab_copy(src, dst, s):
        ncb = src.shape[2] // _CW

        def fn(i, priority):
            r0, c0 = (i // ncb) * 8, (i % ncb) * _CW
            if not isinstance(i, int):
                r0, c0 = pl.multiple_of(r0, 8), pl.multiple_of(c0, _CW)
            rows, cols = pl.ds(r0, 8), pl.ds(c0, _CW)
            _start(src.at[:, rows, cols], dst.at[:, rows, cols], sem.at[s], priority)
        return fn, src.shape[1] // 8 * ncb

    def row_copy(src, dst, s):
        def fn(i, priority):
            rows = pl.ds(pl.multiple_of(i * _FR, _FR), _FR)
            _start(src.at[rows, :], dst.at[rows, :], sem.at[s], priority)
        return fn

    (cp_m, n_m), (cp_q, n_q), (cp_o, n_o) = (slab_copy(wmod_hbm, wmodbuf, _S_M),
                                             slab_copy(wq_hbm, wqbuf, _S_Q),
                                             slab_copy(wo_hbm, wobuf, _S_O))
    split_o = (n_q - _LEAD + n_o - n_m) // 2
    head = ([(cp_m, 0, n_m), (cp_o, 0, split_o)], [(cp_q, _LEAD, n_q), (cp_o, split_o, n_o)])
    cp_u = row_copy(wu_hbm, wubuf, _S_U)
    down_segs = [(row_copy(wd_hbm, wdbuf, _S_D + i), r0 // _FR, (r0 + n) // _FR)
                 for i, (r0, n) in enumerate(pieces)]
    ffn = ([(row_copy(wg_hbm, wgbuf, _S_G), 0, F // _FR), (cp_u, split_u // _FR, F // _FR)]
           + down_segs[:len(wd0)],
           [(cp_u, 0, split_u // _FR)] + down_segs[len(wd0):])

    n_it = W // _ROWS // _UNROLL
    early = int(n_it * _EARLY)

    def issue_kv(kv, p, lo, hi):
        src, dst = ((k_hbm, kbuf), (v_hbm, vbuf))[kv]
        w0 = (NP - 1 if p is None else p) * 2 * _G + _SHIFT

        def copy(z, w, i0, n, r, nr):
            _start(src.at[pl.ds(w, n), pl.ds(Sk - W + r, nr), :],
                   dst.at[z, pl.ds(i0, n), pl.ds(r, nr), :], sem_kv.at[kv, z], z)

        n1 = _G - _SHIFT if p is None else _G

        def rows_at(r, nr):
            copy(0, w0, 0, _G, r, nr)
            copy(1, w0 + _G, 0, n1, r, nr)

        def group(r0, last=False):
            for jj in range(_UNROLL):
                short = last and jj == _UNROLL - 1
                rows_at(r0 + _ROW_OFF + jj * _ROWS, _ROWS - _ROW_OFF if short else _ROWS)
            if p is None:
                copy(1, 0, n1, _SHIFT, r0, _UNROLL * _ROWS)

        if lo == 0:
            rows_at(0, _ROW_OFF)
        _loop(lo, min(hi, n_it - 1),
              lambda i: group(pl.multiple_of(i * _UNROLL * _ROWS, _UNROLL * _ROWS)))
        if hi == n_it:
            group(W - _UNROLL * _ROWS, last=True)

    def head_rows(h):
        return pl.ds(h + _G - _SHIFT, B, stride=H)

    row_w = lax.broadcasted_iota(jnp.int32, (_G, W), 0)
    row_d = lax.broadcasted_iota(jnp.int32, (_G, Dh), 0)
    first, wrap = pl.ds(0, _G), pl.ds(NW, _G)

    for i in range(_LEAD):
        cp_q(i, 1)
    _start(c_hbm, cbuf, sem.at[_S_C], 0)
    _start(x_hbm, xbuf, sem.at[_S_X], 0)
    _issue_streams(head, 0, n_m + _AHEAD)
    _wait_filled(cbuf, sem.at[_S_C])
    _wait_filled(xbuf, sem.at[_S_X])
    _wait_filled(wmodbuf, sem.at[_S_M])
    cf = cbuf[...].astype(_F32)
    sc = (cf * jax.nn.sigmoid(cf)).astype(_BF16)
    xf = xbuf[...].astype(_F32)
    mod = _dot(sc, wmodbuf[...].reshape(D, 6 * D))
    sa, ca, ga, sb, cb, gb = [mod[:, i * D:(i + 1) * D] for i in range(6)]
    h1 = (_layernorm(xf) * (1.0 + ca) + sa).astype(_BF16)
    _issue_streams(head, n_m + _AHEAD)
    issue_kv(0, None, 0, n_it)
    _wait_filled(wqbuf, sem.at[_S_Q])
    _wait_filled(wobuf, sem.at[_S_O])
    q_all = _dot(h1, wqbuf[...].reshape(D, H * Dh))
    zeros = jnp.zeros((_G, Dh), _F32)
    qs[first, :] = zeros
    qs[wrap, :] = zeros
    for h in range(H):
        qs[head_rows(h), :] = q_all[:, h * Dh:(h + 1) * Dh]
    qs[wrap, :] = jnp.where(row_d < _G - _SHIFT, qs[wrap, :], qs[first, :])
    issue_kv(1, None, 0, early)

    def phase_step(t):
        p = (t + NP - 1) % NP
        cur, nxt = jnp.minimum(p, NP - 2), jnp.minimum(t, NP - 2)
        rows = [pl.ds(pl.multiple_of((2 * p + 1 + z) * _G, _G), _G) for z in range(2)]

        def probs(z):
            q = qs[rows[z], :].astype(_BF16)
            _wait_filled(kbuf.at[z], sem_kv.at[0, z])
            s = _dot(q, kbuf[z, 0], _NT)
            for i in range(1, _G):
                s = jnp.where(row_w == i, _dot(q, kbuf[z, i], _NT), s)
            s = s * scale
            e = jnp.exp(s - jnp.max(s, axis=-1, keepdims=True))
            return e.astype(_BF16), jnp.sum(e, axis=-1, keepdims=True)

        def attend(z, e, l):
            _wait_filled(vbuf.at[z], sem_kv.at[1, z])
            o = _dot(e, vbuf[z, 0])
            for i in range(1, _G):
                o = jnp.where(row_d == i, _dot(e, vbuf[z, i]), o)
            ats[rows[z], :] = o / l

        el0 = probs(0)
        pl.when(t == 0)(lambda: issue_kv(1, None, early, n_it))
        pl.when(t > 0)(lambda: issue_kv(1, cur, early, n_it))
        el1 = probs(1)
        pl.when(t < NP - 1)(lambda: issue_kv(0, nxt, 0, early))
        pl.when(t == NP - 1)(lambda: _issue_streams(ffn, 0, _TAIL_FIRST))
        attend(0, *el0)
        pl.when(t < NP - 1)(lambda: issue_kv(0, nxt, early, n_it))
        attend(1, *el1)
        pl.when(t < NP - 1)(lambda: issue_kv(1, nxt, 0, early))

    _loop(0, NP, phase_step)
    _issue_streams(ffn, _TAIL_FIRST)
    ats[first, :] = ats[wrap, :]

    o_all = jnp.concatenate([ats[head_rows(h), :] for h in range(H)], axis=-1).astype(_BF16)
    x1 = xf + ga * _dot(o_all, wobuf[...].reshape(H * Dh, D))
    h2 = (_layernorm(x1) * (1.0 + cb) + sb).astype(_BF16)
    _wait_filled(wgbuf, sem.at[_S_G])
    gate = jax.nn.sigmoid(_dot(h2, wgbuf[...], _NT))
    _wait_filled(wubuf, sem.at[_S_U])
    hh = (gate * _dot(h2, wubuf[...], _NT)).astype(_BF16)
    down = None
    for i, (r0, n) in enumerate(pieces):
        _wait_filled(wdbuf.at[pl.ds(r0, n), :], sem.at[_S_D + i])
        part = _dot(hh[:, r0:r0 + n], wdbuf[pl.ds(r0, n), :])
        down = part if down is None else down + part
    out_ref[...] = (x1 + gb * down).astype(out_ref.dtype)


@jax.jit
def pallas_adaLN_cond__sliding_block_cached__glu_gated_glu__decode_kernel(
    A_x: jax.Array,
    A_k_cache: jax.Array,
    A_v_cache: jax.Array,
    A_wq: jax.Array,
    A_wo: jax.Array,
    B_x: jax.Array,
    B_w_gate: jax.Array,
    B_w_up: jax.Array,
    B_w_down: jax.Array,
    c: jax.Array,
    w_mod: jax.Array,
):
    del B_x
    B, Sq, D = A_x.shape
    _, H, Sk, Dh = A_k_cache.shape
    F = B_w_gate.shape[1]
    W = min(4096, max(256, Sk // 4))
    assert Sq == 1 and A_wq.shape == (D, H * Dh) and B * H % (2 * _G) == 0 and F == 1376
    assert W % (_ROWS * _UNROLL) == 0
    dt = A_x.dtype
    split_u = 1120
    wd0 = ((0, 384),)
    wd1 = ((384, 640), (1024, 256), (1280, 96))

    params = dict(vmem_limit_bytes=48 * 1024 * 1024)
    if hasattr(pltpu.CompilerParams, "disable_semaphore_checks"):
        params["disable_semaphore_checks"] = True

    out = pl.pallas_call(
        functools.partial(_kernel, split_u=split_u, wd0=wd0, wd1=wd1),
        out_shape=jax.ShapeDtypeStruct((B, D), dt),
        in_specs=[pl.BlockSpec(memory_space=pl.ANY)] * 10,
        out_specs=pl.BlockSpec(memory_space=pltpu.VMEM),
        scratch_shapes=[
            pltpu.VMEM((B, D), dt),
            pltpu.VMEM((B, D), dt),
            pltpu.VMEM((_NS, D // _NS, 6 * D), dt),
            pltpu.VMEM((_NS, D // _NS, H * Dh), dt),
            pltpu.VMEM((_NS, H * Dh // _NS, D), dt),
            pltpu.VMEM((2, _G, W, Dh), dt),
            pltpu.VMEM((2, _G, W, Dh), dt),
            pltpu.VMEM((F, D), dt),
            pltpu.VMEM((F, D), dt),
            pltpu.VMEM((F, D), dt),
            pltpu.VMEM((B * H + H + _G, Dh), _F32),
            pltpu.VMEM((B * H + H + _G, Dh), _F32),
            pltpu.SemaphoreType.DMA((2, 2)),
            pltpu.SemaphoreType.DMA((_S_D + len(wd0) + len(wd1),)),
        ],
        compiler_params=pltpu.CompilerParams(**params),
    )(A_x.reshape(B, D), c,
      w_mod.reshape(_NS, D // _NS, 6 * D), A_wq.reshape(_NS, D // _NS, H * Dh),
      A_k_cache.reshape(B * H, Sk, Dh), A_v_cache.reshape(B * H, Sk, Dh),
      A_wo.reshape(_NS, H * Dh // _NS, D), B_w_gate.T, B_w_up.T, B_w_down)
    return out.reshape(B, Sq, D)
```
